```python
import os as _os
_os.environ.setdefault('JAX_PLATFORMS', 'cpu')
import jax
import jax.numpy as jnp

def _softmax(x, axis=-1):
    return jax.nn.softmax(x, axis=axis)

def _gelu(x):
    return jax.nn.gelu(x, approximate=True)

def _silu(x):
    return jax.nn.silu(x)

def _sigmoid(x):
    return jax.nn.sigmoid(x)

def _layernorm(x, axis=-1, eps=1e-05):
    m = jnp.mean(x, axis=axis, keepdims=True)
    v = jnp.var(x, axis=axis, keepdims=True)
    return (x - m) / jnp.sqrt(v + eps)

def _scatter_add(tgt, idx, src, axis=0):
    return tgt.at[idx].add(src)

def _segment_sum(src, seg, n):
    return jax.ops.segment_sum(src, seg, n)

class _Rng:

    def __init__(self, key):
        self._k = key

    def _next(self):
        self._k, sub = jax.random.split(self._k)
        return sub

    def normal(self, shape):
        return jax.random.normal(self._next(), shape, dtype=jnp.bfloat16)

    def randint(self, lo, hi, shape):
        return jax.random.randint(self._next(), shape, lo, hi, dtype=jnp.int32)

    def uniform(self, shape, lo=0.0, hi=1.0):
        return jax.random.uniform(self._next(), shape, jnp.bfloat16, lo, hi)

    def permutation(self, n):
        return jax.random.permutation(self._next(), n)
kernel_name = 'gated_mix__sliding_block__memory_aug_recurrent_mem_tr__prompt'

def setup_inputs():
    _rng = _Rng(jax.random.key(int.from_bytes(__import__("os").urandom(4), "little")))
    _w = lambda a: (lambda t: t.astype(jnp.bfloat16) if jnp.issubdtype(t.dtype, jnp.floating) else t)(jnp.asarray(a))

    def _A_setup():
        B, S, D = (1, 2048, 448)
        return {'x': _w((lambda *s: _rng.normal(s) * 0.05)(B, S, D)), 'wqkv': _w((lambda *s: _rng.normal(s) * 0.8)(D, 3 * D)), 'wo': _w((lambda *s: _rng.normal(s) * 0.05)(D, D))}
    _A_in = _A_setup()

    def _B_setup():
        B, S, Dm = (1, 2048, 448)
        H, Dh = (16, 256)
        M, seg = (8, 32)
        seg = min(seg, S)
        S = S // seg * seg
        return {'x': _w((lambda *s: _rng.normal(s) * 0.05)(B, S, Dm)), 'mem0': _w((lambda *s: _rng.normal(s) * 0.8)(B, M, Dm)), 'Wq': _w((lambda *s: _rng.normal(s) * 3.2)(Dm, H, Dh) * Dm ** (-0.5)), 'Wk': _w((lambda *s: _rng.normal(s) * 3.2)(Dm, H, Dh) * Dm ** (-0.5)), 'Wv': _w((lambda *s: _rng.normal(s) * 0.8)(Dm, H, Dh) * Dm ** (-0.5)), 'Wo': _w((lambda *s: _rng.normal(s) * 0.8)(H, Dh, Dm) * (H * Dh) ** (-0.5)), 'seg_len': seg}
    _B_in = _B_setup()
    return {'A_x': _A_in['x'], 'A_wqkv': _A_in['wqkv'], 'A_wo': _A_in['wo'], 'B_x': _B_in['x'], 'B_mem0': _B_in['mem0'], 'B_Wq': _B_in['Wq'], 'B_Wk': _B_in['Wk'], 'B_Wv': _B_in['Wv'], 'B_Wo': _B_in['Wo'], 'B_seg_len': _B_in['seg_len'], 'gate_w': _w((lambda *s: _rng.normal(s) * 0.05)(448) * 16.0)}

def reference(A_x, A_wqkv, A_wo, B_x, B_mem0, B_Wq, B_Wk, B_Wv, B_Wo, B_seg_len, gate_w):

    def _A_ref(x, wqkv, wo):
        B, S, D = x.shape
        H = 16
        Dh = D // H
        W = 256
        qkv = (lambda x, *d: x.transpose(*d))((x @ wqkv).reshape(B, S, 3, H, Dh), 2, 0, 3, 1, 4)
        q, k, v = (qkv[0], qkv[1], qkv[2])
        scores = jnp.einsum('bhqd,bhkd->bhqk', q, k) * Dh ** (-0.5)
        idx = jnp.arange(S)
        mask = (idx[:, None] - idx[None, :] >= 0) & (idx[:, None] - idx[None, :] < W)
        scores = jnp.where(mask[None, None], scores, -1000000000.0)
        p = _softmax(scores, axis=-1)
        o = jnp.einsum('bhqk,bhkd->bhqd', p, v)
        return (lambda x, *d: x.transpose(*d))(o, 0, 2, 1, 3).reshape(B, S, D) @ wo

    def _B_ref(x, mem0, Wq, Wk, Wv, Wo, seg_len):
        B, S, Dm = x.shape
        H, Dh = (Wq.shape[1], Wq.shape[2])
        M = mem0.shape[1]
        scale = Dh ** (-0.5)
        n_seg = S // seg_len
        L = M + seg_len
        idx = jnp.arange(L)
        mask = (idx[:, None] < M) | (idx[:, None] >= idx[None, :])
        mem = mem0
        outs = []
        for s in range(n_seg):
            xs = x[:, s * seg_len:(s + 1) * seg_len, :].copy()
            h = jnp.concatenate([mem, xs], axis=1)
            q = jnp.einsum('btd,dhe->bhte', h, Wq)
            k = jnp.einsum('btd,dhe->bhte', h, Wk)
            v = jnp.einsum('btd,dhe->bhte', h, Wv)
            scores = jnp.einsum('bhqe,bhke->bhqk', q, k) * scale
            scores = jnp.where(mask[None, None], scores, -1000000000.0)
            p = _softmax(scores, axis=-1)
            o = jnp.einsum('bhqk,bhke->bhqe', p, v)
            o = jnp.einsum('bhte,hed->btd', o, Wo)
            mem = o[:, :M, :].copy()
            outs.append(o[:, M:, :])
        return jnp.concatenate(outs, axis=1)
    x = A_x
    g = _sigmoid((x * gate_w).sum(-1, keepdims=True))
    a = _A_ref(x, A_wqkv, A_wo)
    b = _B_ref(x, B_mem0, B_Wq, B_Wk, B_Wv, B_Wo, B_seg_len)
    return g * a + (1 - g) * b
```

```python
import functools

import jax
import jax.numpy as jnp
import numpy as np
from jax import lax
import jax.experimental.pallas as pl
import jax.experimental.pallas.tpu as pltpu

S = 2048
D = 448
DP = 512
DA = 384
H = 16
NP = H // 2
DH_A = D // H
GA = 4 * DH_A
WIN = 256
DH_B = 256
MEM = 8
SEG = 32
L = MEM + SEG
NJ = L // 8
TB = 128
NB = S // TB
QB = 32
WA = H * DA + NP * 128
NCH = 512
W0 = 512
LOG2E = float(np.log2(np.e))
NEG_B = -1e9 * DH_B ** 0.5

F32 = jnp.float32
BF16 = jnp.bfloat16
U32 = jnp.uint32

SCHEDULE = (
    "T1 T0 G30 R0123 G31 G00 R4567 G01 G02 S31234 G03 G10 G11 S0324 S30 G12 G13 S001 G20 G21 S11234 "
    "G22 G23 S10 U00 U01 S20123 U02 A0 U03 S24 M U10 U11 U12 U13 A1 U20 U21 A2 U22 U23 U30 U31 "
    "Y02134567 O V12 W0 V0 W2341756 V43 Q")

_dot = functools.partial(jnp.dot, preferred_element_type=F32)
_dot_nt = functools.partial(lax.dot_general, dimension_numbers=(((1,), (1,)), ((), ())),
                            preferred_element_type=F32)


def _iota(shape, dim):
    return lax.broadcasted_iota(jnp.int32, shape, dim)


def _rows(xs):
    return jnp.concatenate(xs, axis=0)


def _lanes(xs):
    return jnp.concatenate(xs, axis=1)


def _group(x, k):
    return x[8 * k:8 * k + 8]


def _tile(x, t):
    return x[:, 128 * t:128 * t + 128]


def _roll(v, shift):
    shift %= 128
    return pltpu.roll(v, shift, 1) if shift else v


def _accumulate(old, new):
    return new if old is None else old + new


def _key_allreduce(v, op):
    lane = _iota(v.shape, 1)
    for b in (4, 2, 1):
        v = op(v, jnp.where((lane & b) != 0, _roll(v, b), _roll(v, -b)))
    return v


def _gather_groups(xs, shifts, width):
    n = len(xs)
    lane = _iota(next(x.shape for x in xs if x is not None), 1)

    @functools.cache
    def stage(bit, a):
        if bit == 0:
            return xs[a]
        lo, hi = stage(bit // 2, a), stage(bit // 2, (a + bit) % n)
        if hi is None or lo is None or hi is lo:
            return lo if hi is None else hi
        return jnp.where((lane & (bit * width)) != 0, hi, lo)

    return [stage(n // 2, -s % n) for s in shifts]


def _pair_rows(left, right):
    return [_rows([_group(left, jb), _group(right, jb)]) for jb in range(NJ)]


def _split_tail(y):
    left = _iota(y.shape, 1) < 64
    return _pair_rows(jnp.where(left, y, 0.0), jnp.where(left, 0.0, y))


def _viewers(jb):
    return [ib for ib in range(NJ) if ib == 0 or ib >= jb]


def _b_softmax(body, tail):
    causal = _iota((8, 128), 0) >= (_iota((8, 128), 1) & 7)
    p_body, p_tail = [], []
    for ib in range(NJ):
        jbs = range(NJ) if ib == 0 else range(ib + 1)
        extra = _gather_groups([_group(x, ib) for x in tail], jbs, 16)
        s = [body[ib][jb] + _roll(extra[jb], -16 * jb) for jb in jbs]
        if ib:
            s[ib] = jnp.where(causal, s[ib], NEG_B)
        m = _key_allreduce(functools.reduce(jnp.maximum, s), jnp.maximum)
        e = [jnp.exp2((x - m) * (DH_B ** -0.5 * LOG2E)) for x in s]
        r = 1.0 / _key_allreduce(functools.reduce(jnp.add, e), jnp.add)
        p = [x * r for x in e]
        p_body.append(p)
        rolled = [_roll(x, 16 * jb) for jb, x in enumerate(p)]
        masked = [jnp.zeros((8, 128), F32)] * (NJ - len(p))
        p_tail.append(_gather_groups(rolled + masked + [None] * (NP - NJ), range(NP), 16))
    return p_body, [_rows([p_tail[ib][hp] for ib in range(NJ)]) for hp in range(NP)]


def _kernel(xt_hbm, wqkv_hbm, wo_hbm, mem_hbm, wq_hbm, wk_hbm, wv_hbm, wot_hbm, gw_hbm, out_hbm,
            xt, wqkv0, wqkv1, wo, wq, wk, wv, wot, xn, qt, vt, gate,
            g_body, g_tail, u_body, u_tail, kn, wo_t, keys, values, b_out, a_score, a_prob, out, a_out, a_max, wqkv_t, mem0, gw,
            sem_x, sem_in, sem_out):
    g_body, g_tail, u_body, u_tail, kn, wo_t, keys, values, wqkv_t = [
        r.bitcast(BF16) for r in (g_body, g_tail, u_body, u_tail, kn, wo_t, keys, values, wqkv_t)]

    def cp_x(c):
        cols = pl.ds(pl.multiple_of(c * NCH, NCH), NCH)
        return pltpu.make_async_copy(xt_hbm.at[:, cols], xt.at[:, cols], sem_x.at[c])

    def cp_halves(src, dst, k):
        return [pltpu.make_async_copy(src.at[:, pl.ds(128 * c, 128)], dst.at[c, pl.ds(0, D * H)],
                                      sem_in.at[k + c]) for c in range(2)]

    cp_w0 = pltpu.make_async_copy(wqkv_hbm.at[:, pl.ds(0, W0)], wqkv0.at[pl.ds(0, D)], sem_in.at[0])
    cp_w1 = [pltpu.make_async_copy(wqkv_hbm.at[:, pl.ds(W0, 3 * D - W0)], wqkv1.at[pl.ds(0, D)], sem_in.at[1]),
             pltpu.make_async_copy(gw_hbm, gw, sem_in.at[2]),
             pltpu.make_async_copy(mem_hbm, mem0, sem_in.at[3])]
    cp_qk = cp_halves(wq_hbm, wq, 4) + cp_halves(wk_hbm, wk, 6)
    cp_vo = cp_halves(wv_hbm, wv, 8) + [pltpu.make_async_copy(wot_hbm, wot, sem_in.at[10]),
                                        pltpu.make_async_copy(wo_hbm, wo, sem_in.at[11])]
    cp_w0.start()
    cp_x(0).start()

    wqkv0[pl.ds(D, DP - D), :] = jnp.zeros((DP - D, W0), BF16)
    wqkv1[pl.ds(D, DP - D), :] = jnp.zeros((DP - D, 3 * D - W0), BF16)
    kn[pl.ds(0, WIN), :] = jnp.where((_iota((WIN, DP), 1) & 127) == GA, -1e30, 0.0).astype(BF16)
    vt[:, pl.ds(0, WIN)] = jnp.zeros((D, WIN), F32)
    a_out[...] = jnp.zeros(a_out.shape, F32)
    b_out[...] = jnp.zeros(b_out.shape, F32)

    def load_x(t0):
        x = xt[:, pl.ds(t0, NCH)]
        return _rows([x, x[DA:]])

    def proj_q(t0, x):
        q = _dot(wqkv_t[pl.ds(0, D), :], x) * (DH_A ** -0.5 * LOG2E)
        qt[:, pl.ds(t0, NCH)] = pltpu.bitcast(q.astype(BF16), U32)

    def proj_kv(t0, x):
        xn[pl.ds(t0, NCH), :] = x.astype(F32).T
        k = _dot(wqkv_t[pl.ds(D, D), :], x)
        vg = _dot(wqkv_t[pl.ds(2 * D, D + 16), :], x)
        for g in range(4):
            kg = _rows([k[GA * g:GA * g + GA], jnp.zeros((128 - GA, NCH), F32)])
            kn[pl.ds(WIN + t0, NCH), pl.ds(128 * g, 128)] = kg.T.astype(BF16)
        vt[:, pl.ds(WIN + t0, NCH)] = vg[:D]
        gate[:, pl.ds(t0, NCH)] = jax.nn.sigmoid(vg[D:D + 8])

    cp_w0.wait()
    for c in cp_w1:
        c.start()
    wqkv_t[pl.ds(0, W0), :] = wqkv0[...].T
    cp_x(0).wait()
    cp_x(1).start()
    proj_q(0, load_x(0))
    for c in cp_w1:
        c.wait()
    for c in [cp_x(2), cp_x(3)] + cp_qk:
        c.start()
    wqkv_t[pl.ds(W0, 3 * D - W0), :] = wqkv1[...].T
    gate_rows = jnp.broadcast_to(gw[...].astype(F32).reshape(1, D), (16, D))
    wqkv_t[pl.ds(3 * D, 16), :] = _lanes([gate_rows, jnp.zeros((16, DP - D), F32)]).astype(BF16)
    proj_kv(0, load_x(0))

    def proj_chunk(c, carry):
        cp_x(c).wait()

        @pl.when(c == 2)
        def _():
            for cp in cp_vo:
                cp.start()

        t0 = pl.multiple_of(c * NCH, NCH)
        x = load_x(t0)
        proj_kv(t0, x)
        proj_q(t0, x)
        return carry

    lax.fori_loop(1, S // NCH, proj_chunk, 0)

    def head_pair(buf, hp):
        words = buf.bitcast(U32)
        w = _lanes([words[c, pl.ds(hp, D, stride=NP), :] for c in range(2)])
        return [lax.bitcast_convert_type(x.astype(jnp.uint16), BF16) for x in (w, w >> 16)]

    def fold(value_side, hp, a, b):
        body = u_body if value_side else g_body
        low, side = [], []

        def main(k):
            r = _dot_nt(a[k], b[k][:DA])
            for t in range(3):
                body[:, pl.ds(128 * (H * t + 2 * hp + k), 128)] = _tile(r[:DA], t).astype(BF16)
            low.append(r[DA:])

        def cross(k):
            side.append(_dot_nt(b[k][DA:], a[k][:DA]))

        def corner():
            ta, tb = [_rows([x[DA:] for x in ab]) for ab in (a, b)]
            same_head = (_iota((128, 128), 0) < 64) == (_iota((128, 128), 1) < 64)
            c = jnp.where(same_head, _dot_nt(ta, tb) if value_side else _dot_nt(tb, ta), 0.0).astype(BF16)
            if value_side:
                u_tail[pl.ds(128 * hp, 128), pl.ds(DA, 128)] = c
            else:
                g_tail[pl.ds(DA, 128), pl.ds(128 * hp, 128)] = c

        for k in range(2):
            main(k)
            cross(k)
        corner()
        body[:, pl.ds(128 * (3 * H + hp), 128)] = _rows(side).T.astype(BF16)
        if value_side:
            u_tail[pl.ds(128 * hp, 128), pl.ds(0, DA)] = _rows(low).astype(BF16)
        else:
            g_tail[pl.ds(0, DA), pl.ds(128 * hp, 128)] = _rows(low).T.astype(BF16)

    for c in cp_qk:
        c.wait()
    for hp in range(NP):
        fold(False, hp, head_pair(wk, hp), head_pair(wq, hp))
    for c in cp_vo:
        c.wait()
    for hp in range(NP):
        fold(True, hp, head_pair(wv, hp), (wot[2 * hp], wot[2 * hp + 1]))
    for g in range(4):
        wo_t[:, pl.ds(128 * g, 128)] = _rows([wo[pl.ds(GA * g, GA), :], jnp.zeros((128 - GA, D), BF16)]).T

    def diagonal():
        return _iota((QB, TB), 0) <= (_iota((QB, TB), 1) & (QB - 1))

    def a_scores(i, g):
        q = qt[pl.ds(GA // 2 * g, GA // 2), pl.ds(pl.multiple_of(i * TB, TB), TB)]
        per_head = DH_A // 2
        row = _iota(q.shape, 0)
        head = sum((row >= per_head * k).astype(jnp.int32) for k in range(1, 4))
        rolled = q
        for k in range(1, 4):
            lo, hi = per_head * k // 8 * 8, (per_head * (k + 1) - 1) // 8 * 8 + 8
            part = jnp.where(head[lo:hi] == k, _roll(q[lo:hi], QB * k), rolled[lo:hi])
            rolled = _rows([x for x in (rolled[:lo], part, rolled[hi:]) if x.shape[0]])
        one = jnp.where(_iota((8, TB), 0) == 0, U32(0x3F80), U32(0))
        for u in range(4):
            qu = _rows([jnp.where(_iota(q.shape, 1) >> 5 == ((head + u) & 3), rolled, U32(0)), one])
            k = kn[pl.ds(pl.multiple_of(i * TB + QB * u, QB), WIN + QB), pl.ds(128 * g, 128)]
            s = _dot(k, pltpu.bitcast(qu, BF16))
            s = _rows([jnp.where(diagonal(), s[WIN:], s[:QB]), s[QB:WIN]])
            a_score[:, pl.ds(TB * u, TB)] = s
            a_max[:, pl.ds(TB * u, TB)] = jnp.broadcast_to(jnp.max(s, axis=0, keepdims=True), (8, TB))

    def a_weights(u, c):
        last = WIN // QB
        if not 0 <= c <= last:
            return jnp.zeros((QB // 2, TB), U32)
        cols = pl.ds(TB * u, TB)
        p = jnp.exp2(a_score[pl.ds(QB * (c % last), QB), cols] - _rows([a_max[:, cols]] * (QB // 8)))
        if c == 0:
            p = jnp.where(diagonal(), 0.0, p)
        if c == last:
            p = jnp.where(diagonal(), p, 0.0)
        a_prob.bitcast(BF16)[pl.ds(QB * c, QB), cols] = p.astype(BF16)
        return a_prob[pl.ds(QB // 2 * c, QB // 2), cols]

    def a_values(i, g, kk, acc):
        chunks = [_gather_groups([a_weights(u, cc - u) for u in range(4)], range(4), QB)
                  for cc in range(4 * kk, 4 * kk + 4)]
        row = _iota((32, TB), 0)
        for hh in range(4):
            v = vt[pl.ds(GA * g + DH_A * hh - 4 * (hh % 2), 32), pl.ds(pl.multiple_of((i + kk) * TB, TB), TB)]
            v = jnp.where(row < 4 if hh % 2 else row >= DH_A, 1.0, v)
            acc[hh] = _accumulate(acc[hh], _dot(v, pltpu.bitcast(_rows([c[hh] for c in chunks]), BF16)))

    def a_project(g, acc):
        o = [_roll(x * (1.0 / (x[:1] if hh % 2 else x[31:])), -QB * hh) for hh, x in enumerate(acc)]
        top = _iota((8, TB), 0) < 4
        o = _rows([o[0][:24], jnp.where(top, o[0][24:], o[1][:8]), o[1][8:],
                   o[2][:24], jnp.where(top, o[2][24:], o[3][:8]), o[3][8:],
                   jnp.zeros((128 - GA, TB), F32)]).astype(BF16)
        for c in range(4):
            rows = pl.ds(D // 4 * c, D // 4)
            a = _dot(wo_t[rows, pl.ds(128 * g, 128)], o)
            a_out[rows, :] = a if g == 0 else a_out[rows, :] + a

    def step(i, j, mem):
        h = _rows([mem, xn[pl.ds(pl.multiple_of(i * TB, TB) + SEG * j, SEG), :]])
        h_tail = _split_tail(_tile(h, 3))
        s_body = [[None] * NJ for _ in range(NJ)]
        q_tail, s_tail, y_tail = [None] * NP, [None] * NP, [None] * NP
        o, o_a = [None] * NJ, [None] * 4

        def project(w, z, t, part):
            y = _dot(h[:, :DA], w[:, pl.ds(128 * (H * t + 4 * part), 512)])
            if t < 3:
                pairs = [_pair_rows(_tile(y, k), _tile(y, k + 1)) for k in (0, 2)]
            else:
                pairs = [_split_tail(_tile(y, k)) for k in range(4)]
            for hp, pair in enumerate(pairs, len(pairs) * part):
                for jb in range(NJ):
                    z[pl.ds(128 * jb + 16 * hp, 16), pl.ds(128 * t, 128)] = pair[jb].astype(BF16)

        def tail_keys(hp):
            zero = jnp.zeros((16, 128), F32)
            return _rows([h_tail[(c - hp) % NP] if (c - hp) % NP < NJ else zero for c in range(NP)]).astype(BF16)

        for op in SCHEDULE.split():
            kind, arg = op[0], [int(c) for c in op[1:]]
            if kind == "T":
                y = _dot(h, g_tail[:, pl.ds(512 * arg[0], 512)])
                q_tail[4 * arg[0]:4 * arg[0] + 4] = [_tile(y, k) for k in range(4)]
            elif kind == "G":
                project(g_body, keys, *arg)
            elif kind == "U":
                project(u_body, values, *arg)
            elif kind == "R":
                for hp in arg:
                    s_tail[hp] = _dot_nt(q_tail[hp], tail_keys(hp))
            elif kind == "S":
                t = arg[0]
                for jb in arg[1:]:
                    s = _dot_nt(_rows([_group(_tile(h, t), ib) for ib in _viewers(jb)]),
                                keys[pl.ds(128 * jb, 128), pl.ds(128 * t, 128)])
                    for k, ib in enumerate(_viewers(jb)):
                        s_body[ib][jb] = _accumulate(s_body[ib][jb], _group(s, k))
            elif kind == "M":
                p_body, p_tail = _b_softmax(s_body, s_tail)
            elif kind == "Y":
                for hp in arg:
                    y_tail[hp] = _dot(p_tail[hp], tail_keys(hp))
            elif kind == "V":
                for jb in arg:
                    y = _dot(_rows([p_body[ib][jb] for ib in _viewers(jb)]),
                             values[pl.ds(128 * jb, 128), :])
                    for k, ib in enumerate(_viewers(jb)):
                        o[ib] = _accumulate(o[ib], _group(y, k))
            elif kind == "W":
                for hp in arg:
                    y = _dot(y_tail[hp], u_tail[pl.ds(128 * hp, 128), :])
                    for ib in range(NJ):
                        o[ib] = _accumulate(o[ib], _group(y, ib))
            elif kind == "A":
                a_values(i, j, arg[0], o_a)
            elif kind == "O":
                a_project(j, o_a)
            elif kind == "Q":
                a_scores(*((i, j + 1) if j < 3 else (jnp.minimum(i + 1, NB - 1), 0)))
        o = _rows(o)
        o = _lanes([o[:, :DA], _tile(o, 3) + _roll(_tile(o, 3), 64)])
        b_out[pl.ds(SEG * j, SEG), :] = o[MEM:]
        return o[:MEM]

    def mix(i):
        cols = pl.ds(pl.multiple_of(i * TB, TB), TB)
        g = gate[pl.ds(0, 1), cols]
        out[:, cols] = (g * a_out[...] + (1.0 - g) * b_out[...].T[:D]).astype(BF16)

    def cp_out(i):
        cols = pl.ds(pl.multiple_of(i * TB, TB), TB)
        return pltpu.make_async_copy(out.at[:, cols], out_hbm.at[:, cols], sem_out.at[0])

    def block(i, mem):
        mix(jnp.maximum(i - 1, 0))
        for j in range(TB // SEG):
            mem = step(i, j, mem)

        @pl.when(i > 0)
        def _():
            cp_out(i - 1).start()

        return mem

    m0 = mem0[...].astype(F32)
    a_scores(0, 0)
    lax.fori_loop(0, NB, block, _lanes([m0, m0[:, DA:]]))
    mix(NB - 1)
    cp_out(NB - 1).start()
    pltpu.make_async_copy(out, out_hbm, sem_out.at[0]).wait()


@functools.partial(jax.jit, static_argnames=("B_seg_len",))
def pallas_gated_mix__sliding_block__memory_aug_recurrent_mem_tr__prompt_kernel(
    A_x, A_wqkv, A_wo, B_x, B_mem0, B_Wq, B_Wk, B_Wv, B_Wo, B_seg_len, gate_w,
):
    del B_x
    assert B_seg_len == SEG and A_x.shape == (1, S, D) and B_mem0.shape == (1, MEM, D)
    assert B_Wq.shape == B_Wk.shape == B_Wv.shape == (D, H, DH_B) and A_x.dtype == BF16
    in_hbm = pl.BlockSpec(memory_space=pl.ANY)
    out_t = pl.pallas_call(
        _kernel,
        out_shape=jax.ShapeDtypeStruct((D, S), BF16),
        in_specs=[in_hbm] * 9,
        out_specs=in_hbm,
        scratch_shapes=[
            pltpu.VMEM((D, S), BF16),
            pltpu.VMEM((DP, W0), BF16),
            pltpu.VMEM((DP, 3 * D - W0), BF16),
            pltpu.VMEM((D, D), BF16),
            pltpu.VMEM((2, D * H + 32, 128), BF16),
            pltpu.VMEM((2, D * H + 32, 128), BF16),
            pltpu.VMEM((2, D * H + 32, 128), BF16),
            pltpu.VMEM((H, D, DH_B), BF16),
            pltpu.VMEM((S, DP), F32),
            pltpu.VMEM((D // 2, S), U32),
            pltpu.VMEM((D, WIN + S), F32),
            pltpu.VMEM((8, S), F32),
            pltpu.VMEM((DA // 2, WA), U32),
            pltpu.VMEM((DP // 2, NP * 128), U32),
            pltpu.VMEM((DA // 2, WA), U32),
            pltpu.VMEM((NP * 64, DP), U32),
            pltpu.VMEM(((WIN + S) // 2, DP), U32),
            pltpu.VMEM((D // 2, DP), U32),
            pltpu.VMEM((L * H // 2, DP), U32),
            pltpu.VMEM((L * H // 2, DP), U32),
            pltpu.VMEM((TB, DP), F32),
            pltpu.VMEM((WIN, 4 * TB), F32),
            pltpu.VMEM(((WIN + QB) // 2, 4 * TB), U32),
            pltpu.VMEM((D, S), BF16),
            pltpu.VMEM((D, TB), F32),
            pltpu.VMEM((8, 4 * TB), F32),
            pltpu.VMEM((3 * D // 2 + 8, DP), U32),
            pltpu.VMEM((MEM, D), BF16),
            pltpu.VMEM((D,), BF16),
            pltpu.SemaphoreType.DMA((S // NCH,)),
            pltpu.SemaphoreType.DMA((12,)),
            pltpu.SemaphoreType.DMA((1,)),
        ],
        compiler_params=pltpu.CompilerParams(vmem_limit_bytes=100 * 1024 * 1024),
    )(
        A_x[0].T, A_wqkv, A_wo, B_mem0[0],
        B_Wq.reshape(D * H, DH_B), B_Wk.reshape(D * H, DH_B), B_Wv.reshape(D * H, DH_B),
        B_Wo.transpose(0, 2, 1), gate_w,
    )
    return out_t.T[None]
```

```python
import functools

import jax
import jax.numpy as jnp
import numpy as np
from jax import lax
import jax.experimental.pallas as pl
import jax.experimental.pallas.tpu as pltpu

S = 2048
D = 448
DP = 512
DA = 384
H = 16
NP = H // 2
DH_A = D // H
GA = 4 * DH_A
WIN = 256
DH_B = 256
MEM = 8
SEG = 32
L = MEM + SEG
NJ = L // 8
TB = 128
NB = S // TB
QB = 32
WA = H * DA + NP * 128
N0 = 512
NCH = 768
W0 = 512
LOG2E = float(np.log2(np.e))
NEG_B = -1e9 * DH_B ** 0.5
NEG_A = -1e30

F32 = jnp.float32
BF16 = jnp.bfloat16
U32 = jnp.uint32

SCHEDULE = (
    "T1 T0 G30 G31 R40123 G00 G01 G02 S32134 G03 G10 G11 S0324 S30 G12 G13 S010 G20 G21 S11234 G22 G23 "
    "U00 U01 S20123 U02 S10 S24 U03 M U10 U11 A0 A1 U12 U13 U20 U21 A2 U22 U23 U30 Y02145673 U31 "
    "W0 O V01 W4175632 V342 Q")

_dot = functools.partial(jnp.dot, preferred_element_type=F32)
_dot_nt = functools.partial(lax.dot_general, dimension_numbers=(((1,), (1,)), ((), ())),
                            preferred_element_type=F32)


def _iota(shape, dim):
    return lax.broadcasted_iota(jnp.int32, shape, dim)


def _rows(xs):
    return jnp.concatenate(xs, axis=0)


def _lanes(xs):
    return jnp.concatenate(xs, axis=1)


def _group(x, k):
    return x[8 * k:8 * k + 8]


def _tile(x, t):
    return x[:, 128 * t:128 * t + 128]


def _roll(v, shift):
    shift %= 128
    return pltpu.roll(v, shift, 1) if shift else v


def _accumulate(old, new):
    return new if old is None else old + new


def _key_allreduce(v, op):
    lane = _iota(v.shape, 1)
    for b in (4, 2, 1):
        v = op(v, jnp.where((lane & b) != 0, _roll(v, b), _roll(v, -b)))
    return v


def _gather_groups(xs, shifts, width):
    n = len(xs)
    lane = _iota(next(x.shape for x in xs if x is not None), 1)

    @functools.cache
    def stage(bit, a):
        if bit == 0:
            return xs[a]
        lo, hi = stage(bit // 2, a), stage(bit // 2, (a + bit) % n)
        if hi is None or lo is None or hi is lo:
            return lo if hi is None else hi
        return jnp.where((lane & (bit * width)) != 0, hi, lo)

    return [stage(n // 2, -s % n) for s in shifts]


def _pair_rows(left, right):
    return [_rows([_group(left, jb), _group(right, jb)]) for jb in range(NJ)]


def _split_tail(y):
    left = _iota(y.shape, 1) < 64
    return _pair_rows(jnp.where(left, y, 0.0), jnp.where(left, 0.0, y))


def _viewers(jb):
    return [ib for ib in range(NJ) if ib == 0 or ib >= jb]


def _visible(ib):
    return range(NJ) if ib == 0 else range(ib + 1)


def _transpose_blocks(x):
    row, lane = _iota(x.shape, 0), _iota(x.shape, 1)
    for b in (4, 2, 1):
        up, down = pltpu.roll(x, 8 - b, 0), pltpu.roll(x, b, 0)
        x = jnp.where(((row ^ lane) & b) == 0, x, jnp.where((row & b) != 0, _roll(down, -b), _roll(up, b)))
    return x


def _b_softmax(body, tail):
    causal = _iota((8, 128), 0) >= (_iota((8, 128), 1) & 7)
    p_body, p_tail = [], []
    for ib in range(NJ):
        s = [body[ib][jb] + tail[ib][jb] for jb in _visible(ib)]
        if ib:
            s[ib] = jnp.where(causal, s[ib], NEG_B)
        m = _key_allreduce(functools.reduce(jnp.maximum, s), jnp.maximum)
        e = [jnp.exp2((x - m) * (DH_B ** -0.5 * LOG2E)) for x in s]
        r = 1.0 / _key_allreduce(functools.reduce(jnp.add, e), jnp.add)
        p = [x * r for x in e]
        p_body.append(p)
        rolled = [_roll(x, 16 * jb) for jb, x in enumerate(p)]
        masked = [jnp.zeros((8, 128), F32)] * (NJ - len(p))
        p_tail.append(_gather_groups(rolled + masked + [None] * (NP - NJ), range(NP), 16))
    return p_body, [_rows([p_tail[ib][hp] for ib in range(NJ)]) for hp in range(NP)]


def _kernel(xt_hbm, wqkv_hbm, wo_hbm, mem_hbm, wq_hbm, wk_hbm, wv_hbm, wot_hbm, gw_hbm, out_hbm,
            xt, wqkv0, wqkv1, wo, wq, wk, wv, wot, xn, qt, vt, gate,
            g_body, g_tail, u_body, u_tail, kn, wo_t, keys, values, b_out, a_score, a_prob, out,
            a_out, gw_col, a_max, wqkv_t, mem0, gw, sem_x, sem_in, sem_out):
    g_body, g_tail, u_body, u_tail, kn, wo_t, keys, values, wqkv_t = [
        r.bitcast(BF16) for r in (g_body, g_tail, u_body, u_tail, kn, wo_t, keys, values, wqkv_t)]

    chunks = [(0, N0)] + [(t0, NCH) for t0 in range(N0, S, NCH)]
    cp_x = [pltpu.make_async_copy(xt_hbm.at[:, pl.ds(*c)], xt.at[:, pl.ds(*c)], sem_x.at[k])
            for k, c in enumerate(chunks)]

    def cp_halves(src, dst, k):
        return [pltpu.make_async_copy(src.at[:, pl.ds(128 * c, 128)], dst.at[c, pl.ds(0, D * H)],
                                      sem_in.at[k + c]) for c in range(2)]

    cp_w0 = pltpu.make_async_copy(wqkv_hbm.at[:, pl.ds(0, W0)], wqkv0.at[pl.ds(0, D)], sem_in.at[0])
    cp_w1 = [pltpu.make_async_copy(wqkv_hbm.at[:, pl.ds(W0, 3 * D - W0)], wqkv1.at[pl.ds(0, D)], sem_in.at[1]),
             pltpu.make_async_copy(gw_hbm, gw, sem_in.at[2]),
             pltpu.make_async_copy(mem_hbm, mem0, sem_in.at[3])]
    cp_qk = cp_halves(wq_hbm, wq, 4) + cp_halves(wk_hbm, wk, 6)
    cp_vo = cp_halves(wv_hbm, wv, 8) + [pltpu.make_async_copy(wot_hbm, wot, sem_in.at[10]),
                                        pltpu.make_async_copy(wo_hbm, wo, sem_in.at[11])]
    cp_w0.start()
    cp_x[0].start()

    wqkv0[pl.ds(D, DP - D), :] = jnp.zeros((DP - D, W0), BF16)
    wqkv1[pl.ds(D, DP - D), :] = jnp.zeros((DP - D, 3 * D - W0), BF16)
    kn[pl.ds(0, WIN), :] = jnp.where((_iota((WIN, DP), 1) & 127) == GA, NEG_A, 0.0).astype(BF16)
    vt[:, pl.ds(0, WIN)] = jnp.zeros((D, WIN), F32)
    a_out[...] = jnp.zeros(a_out.shape, F32)
    b_out[...] = jnp.zeros(b_out.shape, F32)

    def load_x(t0, n):
        x = xt[:, pl.ds(t0, n)]
        return _rows([x, x[DA:]])

    def proj_q(t0, x):
        q = _dot(wqkv_t[pl.ds(0, D), :], x) * (DH_A ** -0.5 * LOG2E)
        qt[:, pl.ds(t0, x.shape[1])] = pltpu.bitcast(q.astype(BF16), U32)

    def proj_kv(t0, x):
        n = x.shape[1]
        xf = x.astype(F32)
        xn[pl.ds(t0, n), :] = xf.T
        k = _dot(wqkv_t[pl.ds(D, D), :], x)
        vt[:, pl.ds(WIN + t0, n)] = _dot(wqkv_t[pl.ds(2 * D, D), :], x)
        for g in range(4):
            kg = _rows([k[GA * g:GA * g + GA], jnp.zeros((128 - GA, n), F32)])
            kn[pl.ds(WIN + t0, n), pl.ds(128 * g, 128)] = kg.T.astype(BF16)
        logit = jnp.sum(xf[:D] * _lanes([gw_col[...]] * (n // 128)), axis=0, keepdims=True)
        gate[:, pl.ds(t0, n)] = jnp.broadcast_to(jax.nn.sigmoid(logit), (8, n))

    cp_w0.wait()
    for c in cp_w1:
        c.start()
    wqkv_t[pl.ds(0, W0), :] = wqkv0[...].T
    cp_x[0].wait()
    cp_x[1].start()
    proj_q(0, load_x(0, N0))
    for c in cp_w1:
        c.wait()
    for c in cp_x[2:] + cp_qk:
        c.start()
    wqkv_t[pl.ds(W0, 3 * D - W0), :] = wqkv1[...].T
    gw_col[...] = jnp.broadcast_to(gw[...].astype(F32).reshape(1, D), (128, D)).T
    proj_kv(0, load_x(0, N0))

    for c in cp_x[1:]:
        c.wait()
    for t0, n in chunks[1:]:
        if t0 + n == S:
            for c in cp_vo:
                c.start()
        x = load_x(t0, n)
        proj_kv(t0, x)
        proj_q(t0, x)

    def head_pair(buf, hp):
        words = buf.bitcast(U32)
        w = _lanes([words[c, pl.ds(hp, D, stride=NP), :] for c in range(2)])
        return [lax.bitcast_convert_type(x.astype(jnp.uint16), BF16) for x in (w, w >> 16)]

    def fold(value_side, hp, a, b):
        body = u_body if value_side else g_body
        low, side = [], []
        for k in range(2):
            r = _dot_nt(a[k], b[k][:DA])
            for t in range(3):
                body[:, pl.ds(128 * (H * t + 2 * hp + k), 128)] = _tile(r[:DA], t).astype(BF16)
            low.append(r[DA:])
            side.append(_dot_nt(b[k][DA:], a[k][:DA]))
        a_tail, b_tail = [_rows([x[DA:] for x in ab]) for ab in (a, b)]
        same_head = (_iota((128, 128), 0) < 64) == (_iota((128, 128), 1) < 64)
        corner = _dot_nt(a_tail, b_tail) if value_side else _dot_nt(b_tail, a_tail)
        corner = jnp.where(same_head, corner, 0.0).astype(BF16)
        body[:, pl.ds(128 * (3 * H + hp), 128)] = _rows(side).T.astype(BF16)
        if value_side:
            u_tail[pl.ds(128 * hp, 128), pl.ds(DA, 128)] = corner
            u_tail[pl.ds(128 * hp, 128), pl.ds(0, DA)] = _rows(low).astype(BF16)
        else:
            g_tail[pl.ds(DA, 128), pl.ds(128 * hp, 128)] = corner
            g_tail[pl.ds(0, DA), pl.ds(128 * hp, 128)] = _rows(low).T.astype(BF16)

    for c in cp_qk:
        c.wait()
    for hp in range(NP):
        fold(False, hp, head_pair(wk, hp), head_pair(wq, hp))
    for c in cp_vo:
        c.wait()
    for hp in range(NP):
        fold(True, hp, head_pair(wv, hp), (wot[2 * hp], wot[2 * hp + 1]))
    for g in range(4):
        wo_t[:, pl.ds(128 * g, 128)] = _rows([wo[pl.ds(GA * g, GA), :], jnp.zeros((128 - GA, D), BF16)]).T

    def diagonal():
        return _iota((QB, TB), 0) <= (_iota((QB, TB), 1) & (QB - 1))

    def a_scores(i, g, first=False):
        q = qt[pl.ds(GA // 2 * g, GA // 2), pl.ds(pl.multiple_of(i * TB, TB), TB)]
        per_head = DH_A // 2
        row = _iota(q.shape, 0)
        head = sum((row >= per_head * k).astype(jnp.int32) for k in range(1, 4))
        rolled = q
        for k in range(1, 4):
            lo, hi = per_head * k // 8 * 8, (per_head * (k + 1) - 1) // 8 * 8 + 8
            part = jnp.where(head[lo:hi] == k, _roll(q[lo:hi], QB * k), rolled[lo:hi])
            rolled = _rows([x for x in (rolled[:lo], part, rolled[hi:]) if x.shape[0]])
        one = jnp.where(_iota((8, TB), 0) == 0, np.uint32(0x3F80), np.uint32(0))
        for u in range(4):
            qu = _rows([jnp.where(_iota(q.shape, 1) >> 5 == ((head + u) & 3), rolled, np.uint32(0)), one])
            skip = WIN - QB * u if first else 0
            k = kn[pl.ds(pl.multiple_of(i * TB + QB * u + skip, QB), WIN + QB - skip), pl.ds(128 * g, 128)]
            s = _dot(k, pltpu.bitcast(qu, BF16))
            if first:
                s = _rows([jnp.full((skip, TB), NEG_A, F32), s])
            s = _rows([jnp.where(diagonal(), s[WIN:], s[:QB]), s[QB:WIN]])
            a_score[:, pl.ds(TB * u, TB)] = s
            a_max[:, pl.ds(TB * u, TB)] = jnp.broadcast_to(jnp.max(s, axis=0, keepdims=True), (8, TB))

    def a_weights(u, c):
        last = WIN // QB
        if not 0 <= c <= last:
            return jnp.zeros((QB // 2, TB), U32)
        cols = pl.ds(TB * u, TB)
        p = jnp.exp2(a_score[pl.ds(QB * (c % last), QB), cols] - _rows([a_max[:, cols]] * (QB // 8)))
        if c == 0:
            p = jnp.where(diagonal(), 0.0, p)
        if c == last:
            p = jnp.where(diagonal(), p, 0.0)
        a_prob.bitcast(BF16)[pl.ds(QB * c, QB), cols] = p.astype(BF16)
        return a_prob[pl.ds(QB // 2 * c, QB // 2), cols]

    def a_values(i, g, kk, acc):
        p = [_gather_groups([a_weights(u, cc - u) for u in range(4)], range(4), QB)
             for cc in range(4 * kk, 4 * kk + 4)]
        row = _iota((32, TB), 0)
        for hh in range(4):
            v = vt[pl.ds(GA * g + DH_A * hh - 4 * (hh % 2), 32), pl.ds(pl.multiple_of((i + kk) * TB, TB), TB)]
            v = jnp.where(row < 4 if hh % 2 else row >= DH_A, 1.0, v)
            acc[hh] = _accumulate(acc[hh], _dot(v, pltpu.bitcast(_rows([c[hh] for c in p]), BF16)))

    def a_project(g, acc):
        o = [_roll(x * (1.0 / (x[:1] if hh % 2 else x[31:])), -QB * hh) for hh, x in enumerate(acc)]
        top = _iota((8, TB), 0) < 4
        o = _rows([o[0][:24], jnp.where(top, o[0][24:], o[1][:8]), o[1][8:],
                   o[2][:24], jnp.where(top, o[2][24:], o[3][:8]), o[3][8:],
                   jnp.zeros((128 - GA, TB), F32)]).astype(BF16)
        for c in range(4):
            rows = pl.ds(D // 4 * c, D // 4)
            a = _dot(wo_t[rows, pl.ds(128 * g, 128)], o)
            a_out[rows, :] = a if g == 0 else a_out[rows, :] + a

    def step(i, j, mem):
        h = _rows([mem, xn[pl.ds(pl.multiple_of(i * TB, TB) + SEG * j, SEG), :]])
        h_tail = _split_tail(_tile(h, 3))
        s_body, s_tail = [[[None] * NJ for _ in range(NJ)] for _ in range(2)]
        q_tail, y_tail = [None] * NP, [None] * NP
        o, o_a = [None] * NJ, [None] * 4

        def project(w, z, t, part):
            y = _dot(h[:, :DA], w[:, pl.ds(128 * (H * t + 4 * part), 512)])
            if t < 3:
                pairs = [_pair_rows(_tile(y, k), _tile(y, k + 1)) for k in (0, 2)]
            else:
                pairs = [_split_tail(_tile(y, k)) for k in range(4)]
            for hp, pair in enumerate(pairs, len(pairs) * part):
                for jb in range(NJ):
                    z[pl.ds(128 * jb + 16 * hp, 16), pl.ds(128 * t, 128)] = pair[jb].astype(BF16)

        def tail_keys(hp):
            zero = jnp.zeros((16, 128), F32)
            return _rows([h_tail[(c - hp) % NP] if (c - hp) % NP < NJ else zero for c in range(NP)]).astype(BF16)

        for op in SCHEDULE.split():
            kind, arg = op[0], [int(c) for c in op[1:]]
            if kind == "T":
                y = _dot(h, g_tail[:, pl.ds(512 * arg[0], 512)])
                q_tail[4 * arg[0]:4 * arg[0] + 4] = [_split_tail(_tile(y, k)) for k in range(4)]
            elif kind == "G":
                project(g_body, keys, *arg)
            elif kind == "U":
                project(u_body, values, *arg)
            elif kind == "R":
                for ib in arg:
                    s = _dot_nt(_tile(h, 3)[:8 * len(_visible(ib))], _rows([z[ib] for z in q_tail]).astype(BF16))
                    for jb in _visible(ib):
                        s_tail[ib][jb] = _transpose_blocks(_group(s, jb))
            elif kind == "S":
                t = arg[0]
                for jb in arg[1:]:
                    s = _dot_nt(_rows([_group(_tile(h, t), ib) for ib in _viewers(jb)]),
                                keys[pl.ds(128 * jb, 128), pl.ds(128 * t, 128)])
                    for k, ib in enumerate(_viewers(jb)):
                        s_body[ib][jb] = _accumulate(s_body[ib][jb], _group(s, k))
            elif kind == "M":
                p_body, p_tail = _b_softmax(s_body, s_tail)
            elif kind == "Y":
                for hp in arg:
                    y_tail[hp] = _dot(p_tail[hp], tail_keys(hp))
            elif kind == "V":
                for jb in arg:
                    y = _dot(_rows([p_body[ib][jb] for ib in _viewers(jb)]),
                             values[pl.ds(128 * jb, 128), :])
                    for k, ib in enumerate(_viewers(jb)):
                        o[ib] = _accumulate(o[ib], _group(y, k))
            elif kind == "W":
                for hp in arg:
                    y = _dot(y_tail[hp], u_tail[pl.ds(128 * hp, 128), :])
                    for ib in range(NJ):
                        o[ib] = _accumulate(o[ib], _group(y, ib))
            elif kind == "A":
                a_values(i, j, arg[0], o_a)
            elif kind == "O":
                a_project(j, o_a)
            elif kind == "Q":
                a_scores(*((i, j + 1) if j < 3 else (jnp.minimum(i + 1, NB - 1), 0)))
        o = _rows(o)
        o = _lanes([o[:, :DA], _tile(o, 3) + _roll(_tile(o, 3), 64)])
        b_out[pl.ds(SEG * j, SEG), :] = o[MEM:]
        return o[:MEM]

    def mix(i):
        cols = pl.ds(pl.multiple_of(i * TB, TB), TB)
        g = gate[pl.ds(0, 1), cols]
        out[:, cols] = (g * a_out[...] + (1.0 - g) * b_out[...].T[:D]).astype(BF16)

    def cp_out(i):
        cols = pl.ds(pl.multiple_of(i * TB, TB), TB)
        return pltpu.make_async_copy(out.at[:, cols], out_hbm.at[:, cols], sem_out.at[0])

    def block(i, mem):
        mix(jnp.maximum(i - 1, 0))
        for j in range(TB // SEG):
            mem = step(i, j, mem)

        @pl.when(i > 0)
        def _():
            cp_out(i - 1).start()

        return mem

    m0 = mem0[...].astype(F32)
    a_scores(0, 0, first=True)
    lax.fori_loop(0, NB, block, _lanes([m0, m0[:, DA:]]))
    mix(NB - 1)
    cp_out(NB - 1).start()
    pltpu.make_async_copy(out, out_hbm, sem_out.at[0]).wait()


@functools.partial(jax.jit, static_argnames=("B_seg_len",))
def pallas_gated_mix__sliding_block__memory_aug_recurrent_mem_tr__prompt_kernel(
    A_x, A_wqkv, A_wo, B_x, B_mem0, B_Wq, B_Wk, B_Wv, B_Wo, B_seg_len, gate_w,
):
    del B_x
    assert B_seg_len == SEG and A_x.shape == (1, S, D) and B_mem0.shape == (1, MEM, D)
    assert B_Wq.shape == B_Wk.shape == B_Wv.shape == (D, H, DH_B) and A_x.dtype == BF16
    in_hbm = pl.BlockSpec(memory_space=pl.ANY)
    out_t = pl.pallas_call(
        _kernel,
        out_shape=jax.ShapeDtypeStruct((D, S), BF16),
        in_specs=[in_hbm] * 9,
        out_specs=in_hbm,
        scratch_shapes=[
            pltpu.VMEM((D, S), BF16),
            pltpu.VMEM((DP, W0), BF16),
            pltpu.VMEM((DP, 3 * D - W0), BF16),
            pltpu.VMEM((D, D), BF16),
            pltpu.VMEM((2, D * H + 32, 128), BF16),
            pltpu.VMEM((2, D * H + 32, 128), BF16),
            pltpu.VMEM((2, D * H + 32, 128), BF16),
            pltpu.VMEM((H, D, DH_B), BF16),
            pltpu.VMEM((S, DP), F32),
            pltpu.VMEM((D // 2, S), U32),
            pltpu.VMEM((D, WIN + S), F32),
            pltpu.VMEM((8, S), F32),
            pltpu.VMEM((DA // 2, WA), U32),
            pltpu.VMEM((DP // 2, NP * 128), U32),
            pltpu.VMEM((DA // 2, WA), U32),
            pltpu.VMEM((NP * 64, DP), U32),
            pltpu.VMEM(((WIN + S) // 2, DP), U32),
            pltpu.VMEM((D // 2, DP), U32),
            pltpu.VMEM((L * H // 2, DP), U32),
            pltpu.VMEM((L * H // 2, DP), U32),
            pltpu.VMEM((TB, DP), F32),
            pltpu.VMEM((WIN, 4 * TB), F32),
            pltpu.VMEM(((WIN + QB) // 2, 4 * TB), U32),
            pltpu.VMEM((D, S), BF16),
            pltpu.VMEM((D, TB), F32),
            pltpu.VMEM((D, 128), F32),
            pltpu.VMEM((8, 4 * TB), F32),
            pltpu.VMEM((3 * D // 2, DP), U32),
            pltpu.VMEM((MEM, D), BF16),
            pltpu.VMEM((D,), BF16),
            pltpu.SemaphoreType.DMA((1 + (S - N0) // NCH,)),
            pltpu.SemaphoreType.DMA((12,)),
            pltpu.SemaphoreType.DMA((1,)),
        ],
        compiler_params=pltpu.CompilerParams(vmem_limit_bytes=100 * 1024 * 1024),
    )(
        A_x[0].T, A_wqkv, A_wo, B_mem0[0],
        B_Wq.reshape(D * H, DH_B), B_Wk.reshape(D * H, DH_B), B_Wv.reshape(D * H, DH_B),
        B_Wo.transpose(0, 2, 1), gate_w,
    )
    return out_t.T[None]
```
